```python
import os as _os
_os.environ.setdefault('JAX_PLATFORMS', 'cpu')
import jax
import jax.numpy as jnp

def _softmax(x, axis=-1):
    return jax.nn.softmax(x, axis=axis)

def _gelu(x):
    return jax.nn.gelu(x, approximate=True)

def _silu(x):
    return jax.nn.silu(x)

def _sigmoid(x):
    return jax.nn.sigmoid(x)

def _layernorm(x, axis=-1, eps=1e-05):
    m = jnp.mean(x, axis=axis, keepdims=True)
    v = jnp.var(x, axis=axis, keepdims=True)
    return (x - m) / jnp.sqrt(v + eps)

def _scatter_add(tgt, idx, src, axis=0):
    return tgt.at[idx].add(src)

def _segment_sum(src, seg, n):
    return jax.ops.segment_sum(src, seg, n)

class _Rng:

    def __init__(self, key):
        self._k = key

    def _next(self):
        self._k, sub = jax.random.split(self._k)
        return sub

    def normal(self, shape):
        return jax.random.normal(self._next(), shape, dtype=jnp.bfloat16)

    def randint(self, lo, hi, shape):
        return jax.random.randint(self._next(), shape, lo, hi, dtype=jnp.int32)

    def uniform(self, shape, lo=0.0, hi=1.0):
        return jax.random.uniform(self._next(), shape, jnp.bfloat16, lo, hi)

    def permutation(self, n):
        return jax.random.permutation(self._next(), n)
kernel_name = 'sequential_preLN__memory_aug_recurrent_mem_tr__swiglu_ffn__prompt'

def setup_inputs():
    _rng = _Rng(jax.random.key(int.from_bytes(__import__("os").urandom(4), "little")))
    _w = lambda a: (lambda t: t.astype(jnp.bfloat16) if jnp.issubdtype(t.dtype, jnp.floating) else t)(jnp.asarray(a))

    def _A_setup():
        B, S, Dm = (1, 2048, 640)
        H, Dh = (32, 192)
        M, seg = (8, 32)
        seg = min(seg, S)
        S = S // seg * seg
        return {'x': _w((lambda *s: _rng.normal(s) * 0.05)(B, S, Dm)), 'mem0': _w((lambda *s: _rng.normal(s) * 0.1)(B, M, Dm)), 'Wq': _w((lambda *s: _rng.normal(s) * 1.6)(Dm, H, Dh) * Dm ** (-0.5)), 'Wk': _w((lambda *s: _rng.normal(s) * 1.6)(Dm, H, Dh) * Dm ** (-0.5)), 'Wv': _w((lambda *s: _rng.normal(s) * 0.1)(Dm, H, Dh) * Dm ** (-0.5)), 'Wo': _w((lambda *s: _rng.normal(s) * 0.1)(H, Dh, Dm) * (H * Dh) ** (-0.5)), 'seg_len': seg}
    _A_in = _A_setup()

    def _B_setup():
        B, S, D, F = (1, 2048, 640, 1536)
        return {'x': _w((lambda *s: _rng.normal(s) * 0.05)(B, S, D)), 'w_gate': _w((lambda *s: _rng.normal(s) * 0.05)(D, F)), 'w_up': _w((lambda *s: _rng.normal(s) * 0.05)(D, F)), 'w_down': _w((lambda *s: _rng.normal(s) * 0.05)(F, D))}
    _B_in = _B_setup()
    return {'A_x': _A_in['x'], 'A_mem0': _A_in['mem0'], 'A_Wq': _A_in['Wq'], 'A_Wk': _A_in['Wk'], 'A_Wv': _A_in['Wv'], 'A_Wo': _A_in['Wo'], 'A_seg_len': _A_in['seg_len'], 'B_x': _B_in['x'], 'B_w_gate': _B_in['w_gate'], 'B_w_up': _B_in['w_up'], 'B_w_down': _B_in['w_down']}

def reference(A_x, A_mem0, A_Wq, A_Wk, A_Wv, A_Wo, A_seg_len, B_x, B_w_gate, B_w_up, B_w_down):

    def _A_ref(x, mem0, Wq, Wk, Wv, Wo, seg_len):
        B, S, Dm = x.shape
        H, Dh = (Wq.shape[1], Wq.shape[2])
        M = mem0.shape[1]
        scale = Dh ** (-0.5)
        n_seg = S // seg_len
        L = M + seg_len
        idx = jnp.arange(L)
        mask = (idx[:, None] < M) | (idx[:, None] >= idx[None, :])
        mem = mem0
        outs = []
        for s in range(n_seg):
            xs = x[:, s * seg_len:(s + 1) * seg_len, :].copy()
            h = jnp.concatenate([mem, xs], axis=1)
            q = jnp.einsum('btd,dhe->bhte', h, Wq)
            k = jnp.einsum('btd,dhe->bhte', h, Wk)
            v = jnp.einsum('btd,dhe->bhte', h, Wv)
            scores = jnp.einsum('bhqe,bhke->bhqk', q, k) * scale
            scores = jnp.where(mask[None, None], scores, -1000000000.0)
            p = _softmax(scores, axis=-1)
            o = jnp.einsum('bhqk,bhke->bhqe', p, v)
            o = jnp.einsum('bhte,hed->btd', o, Wo)
            mem = o[:, :M, :].copy()
            outs.append(o[:, M:, :])
        return jnp.concatenate(outs, axis=1)

    def _B_ref(x, w_gate, w_up, w_down):
        g = _silu(x @ w_gate)
        u = x @ w_up
        return g * u @ w_down
    x = A_x
    h = x + _A_ref(_layernorm(x, axis=-1), A_mem0, A_Wq, A_Wk, A_Wv, A_Wo, A_seg_len)
    h2 = h + _B_ref(_layernorm(h, axis=-1), B_w_gate, B_w_up, B_w_down)
    return h2
```

```python
import functools

import jax
import jax.numpy as jnp
import jax.experimental.pallas as pl
import jax.experimental.pallas.tpu as pltpu

F32 = jnp.float32
BF16 = jnp.bfloat16
U32 = jnp.uint32
NN = (((1,), (0,)), ((), ()))
NT = (((1,), (1,)), ((), ()))
EPS = 1e-5
LANES = 128
PRE_COLS = (384, 384, 128)
NSTAGE = 4
UNROLL = 4
G = 2
SPC = 16


def _dot(a, b, dims=NN):
    return jax.lax.dot_general(a, b, dims, preferred_element_type=F32)


def _ln(x):
    m = jnp.mean(x, axis=-1, keepdims=True)
    c = x - m
    v = jnp.mean(c * c, axis=-1, keepdims=True)
    return c / jnp.sqrt(v + EPS)


def _schedule(n):
    prog = [("down", 0)]
    for i in range(n):
        for name, lag in (("q", 0), ("v", 0), ("k", 0), ("scores", 1), ("pv", 2), ("wo", 3)):
            if i >= lag:
                prog.append((name, i - lag))
        if i == 6:
            prog.append(("ln_h", 0))
        if i == 9:
            prog.append(("ln_x", 0))
    return prog + [("scores", n - 1), ("wo", n - 3), ("gate", 0), ("pv", n - 2), ("up", 0),
                   ("pv", n - 1), ("wo", n - 2), ("wo", n - 1)]


def _kernel(x_hbm, mem0_hbm, wq_hbm, wk_hbm, wv_hbm, wo_hbm, wg_hbm, wu_hbm, wd_hbm,
            out_hbm,
            x_ref, xt_ref, xn_ref, stage_ref, wqkv_ref, wo_ref, wg_ref, wu_ref, wd_ref,
            pre_ref, h_ref, hn_ref, act_ref, facc_ref, out_ref, mem0_ref,
            sem_mem, sem_xt, sem_xh, sem_stage, sem_wo, sem_ffn, sem_out,
            *, S, D, H, Dh, M, seg, F):
    NP = H // 2
    PW = 2 * Dh
    L = M + seg
    n_seg = S // seg
    n_iter = n_seg // UNROLL
    GR = G * seg
    n_grp = S // GR
    FQ = F // G
    XH = seg - M
    PC = sum(PRE_COLS)
    scale = Dh ** (-0.5)

    mem_copy = pltpu.make_async_copy(mem0_hbm, mem0_ref, sem_mem)

    def tail_copy(i):
        segs = pl.ds(i * SPC, SPC)
        return pltpu.make_async_copy(x_hbm.at[segs, XH:, :], x_ref.at[segs, XH:, :], sem_xt.at[i])

    def head_copy(i):
        segs = pl.ds(i * UNROLL, UNROLL)
        return pltpu.make_async_copy(x_hbm.at[segs, :XH, :], x_ref.at[segs, :XH, :], sem_xh.at[i % 2])

    def stage_copy(p, i):
        rows = pl.ds(pl.multiple_of(p * PW, PW), PW)
        return pltpu.make_async_copy((wq_hbm, wk_hbm, wv_hbm)[i].at[rows, :],
                                     stage_ref.at[p % NSTAGE, i], sem_stage.at[p % NSTAGE, i])

    def wo_copy(p):
        rows = pl.ds(pl.multiple_of(p * PW, PW), PW)
        return pltpu.make_async_copy(wo_hbm.at[rows, :], wo_ref.at[p], sem_wo.at[p])

    def ffn_copies():
        cs = []
        for j in range(G):
            part = pl.ds(j * FQ, FQ)
            cs += [pltpu.make_async_copy(wg_hbm.at[:, part], wg_ref.at[j], sem_ffn.at[0, j]),
                   pltpu.make_async_copy(wu_hbm.at[:, part], wu_ref.at[j], sem_ffn.at[1, j]),
                   pltpu.make_async_copy(wd_hbm.at[part, :], wd_ref.at[j], sem_ffn.at[2, j])]
        return cs

    def out_copy(g):
        rows = pl.ds(pl.multiple_of(g * GR, GR), GR)
        return pltpu.make_async_copy(out_ref.at[rows, :], out_hbm.at[rows, :], sem_out.at[g])

    for i in range(n_seg // SPC):
        tail_copy(i).start()
    for ref in (h_ref, hn_ref, act_ref, facc_ref):
        ref[...] = jnp.zeros(ref.shape, ref.dtype)

    def ln_tails(i, c):
        tail_copy(i).wait()

        @pl.when(i == 0)
        def _():
            stage_copy(0, 0).start()

        @pl.when(i == 2)
        def _():
            stage_copy(0, 1).start()
            stage_copy(0, 2).start()

        xs = x_ref[pl.ds(i * SPC, SPC), XH:, :].astype(F32).reshape(SPC * M, D)
        xt_ref[pl.ds(pl.multiple_of(i * SPC * M, SPC * M), SPC * M), :] = _ln(xs)
        return c
    jax.lax.fori_loop(0, n_seg // SPC, ln_tails, 0)

    def take(p, i):
        w = stage_ref[p % NSTAGE, i]
        wqkv_ref[3 * p + i] = pltpu.bitcast(w.T, U32)
        if PRE_COLS[i]:
            col = pl.multiple_of(p * PC + sum(PRE_COLS[:i]), LANES)
            pre_ref[:, pl.ds(col, PRE_COLS[i])] = _dot(xt_ref[...], w[:PRE_COLS[i]], NT)

    stage_copy(0, 0).wait()
    for i in range(3):
        stage_copy(1, i).start()
    take(0, 0)
    for i in (1, 2):
        stage_copy(0, i).wait()
    for p in range(2, NSTAGE):
        for i in range(3):
            stage_copy(p, i).start()
    for c in (wo_copy(0), wo_copy(1), head_copy(0), head_copy(1), mem_copy):
        c.start()
    for i in (1, 2):
        take(0, i)

    def pre_body(p, c):
        for i in range(3):
            stage_copy(p, i).wait()
        take(p, 0)

        @pl.when(p + 1 < NP)
        def _():
            wo_copy(p + 1).start()

        for n, cp in enumerate(ffn_copies()):
            pl.when(p == 2 * n + 2)(cp.start)

        @pl.when(p + NSTAGE - 1 < NP)
        def _():
            for i in range(3):
                stage_copy(p + NSTAGE - 1, i).start()

        for i in (1, 2):
            take(p, i)
        return c
    jax.lax.fori_loop(1, NP, pre_body, 0)
    for p in range(NP):
        wo_copy(p).wait()
    head_copy(0).wait()
    mem_copy.wait()
    for c in ffn_copies():
        c.wait()

    def ln_x(s, slot):
        xn_ref[slot] = _ln(x_ref[jnp.minimum(s, n_seg - 1)].astype(F32))

    def ffn_stages(s):
        g, j = s // G, s % G
        t = jnp.maximum(s - 1, 0)
        gd, jd = t // G, t % G
        st = {}

        def ln_h(_):
            rows = pl.ds(pl.multiple_of(jd * seg, seg), seg)
            hn_ref[gd % 2, rows, :] = _ln(h_ref[gd % 2, rows, :])

        def gate(_):
            st["gate"] = _dot(hn_ref[(g + 1) % 2], wg_ref[j])

        def up(_):
            a = st.pop("gate")
            act_ref[...] = a * jax.nn.sigmoid(a) * _dot(hn_ref[(g + 1) % 2], wu_ref[j])

        def down(_):
            res = (jnp.where(jd == 0, h_ref[(gd + 1) % 2], facc_ref[...])
                   + _dot(act_ref[...], wd_ref[jd]))
            facc_ref[...] = res
            rows = pl.ds(pl.multiple_of(jnp.maximum(gd - 1, 0) * GR, GR), GR)
            out_ref[rows, :] = res.astype(out_ref.dtype)

        def write(_):
            @pl.when((jd == G - 1) & (gd > 0))
            def _():
                out_copy(gd - 1).start()

        return dict(ln_h=ln_h, gate=gate, up=up, down=down, write=write)

    def step(s, u, mem):
        row = jax.lax.broadcasted_iota(jnp.int32, (L, LANES), 0)
        lane = jax.lax.broadcasted_iota(jnp.int32, (L, LANES), 1)
        first = lane < L
        real = lane < 2 * L
        key = jnp.where(first, lane, lane - L)
        visible = real & ((row < M) | (row >= key))
        fill = jnp.where(real, -1000000000.0, -jnp.inf).astype(F32)
        low = lane < Dh - LANES

        h = jnp.concatenate([mem, xn_ref[u % 2]], axis=0)
        tail_rows = pl.ds(pl.multiple_of(s * M, M), M)

        def project(i):
            n = PRE_COLS[i % 3]
            col = (i // 3) * PC + sum(PRE_COLS[:i % 3])
            parts = []
            if n:
                y = _dot(h[:M + XH], pltpu.bitcast(wqkv_ref[i, :, :n], BF16))
                parts.append(jnp.concatenate([y, pre_ref[tail_rows, col:col + n]], axis=0))
            if n < PW:
                parts.append(_dot(h, pltpu.bitcast(wqkv_ref[i, :, n:], BF16)))
            return jnp.concatenate(parts, axis=1)

        def stack(t):
            t0, t1, t2 = t[:, :LANES], t[:, LANES:2 * LANES], t[:, 2 * LANES:]
            z8 = jnp.zeros((8, LANES), F32)
            zb = lambda n: jnp.zeros((n, LANES), BF16)
            c0 = [jnp.concatenate([t0, z8], axis=0).astype(BF16), zb(LANES - L - 8)]
            c1 = [jnp.concatenate([jnp.where(low, t1, 0.0), jnp.where(low, 0.0, t1)],
                                  axis=0).astype(BF16), zb(LANES - 2 * L)]
            c2 = [zb(L - 8), jnp.concatenate([z8, t2], axis=0).astype(BF16), zb(LANES - 2 * L)]
            return jnp.concatenate([jnp.concatenate(c, axis=0) for c in (c0, c1, c2)], axis=1)

        st = {}

        def q(p):
            st["q", p] = project(3 * p)

        def k(p):
            st["k", p] = stack(project(3 * p + 1))

        def v(p):
            st["v", p] = stack(project(3 * p + 2))

        def scores(p):
            t = jnp.where(visible, _dot(st.pop(("q", p)), st.pop(("k", p)), NT) * scale, fill)
            m_a = jnp.max(jnp.where(first, t, -jnp.inf), axis=-1, keepdims=True)
            m_b = jnp.max(jnp.where(first, -jnp.inf, t), axis=-1, keepdims=True)
            e = jnp.exp(t - jnp.where(first, m_a, m_b))
            l_a = jnp.sum(jnp.where(first, e, 0.0), axis=-1, keepdims=True)
            l_b = jnp.sum(jnp.where(first, 0.0, e), axis=-1, keepdims=True)
            st["p", p] = e / jnp.where(first, l_a, l_b)

        def pv(p):
            st["o", p] = _dot(st.pop(("p", p)), st.pop(("v", p)))

        def wo(p):
            d = _dot(st.pop(("o", p)), wo_ref[p])
            st["acc"] = d if p == 0 else st["acc"] + d

        stages = dict(q=q, k=k, v=v, scores=scores, pv=pv, wo=wo,
                      ln_x=lambda _: ln_x(s + 1, (u + 1) % 2), **ffn_stages(s))
        for name, p in _schedule(NP):
            stages[name](p)
        acc = st["acc"]
        rows = pl.ds(pl.multiple_of((s % G) * seg, seg), seg)
        h_ref[(s // G) % 2, rows, :] = x_ref[s].astype(F32) + acc[M:, :]
        stages["write"](0)
        return acc[:M, :]

    def iteration(i, mem):
        @pl.when(i + 1 < n_iter)
        def _():
            head_copy(i + 1).wait()

        @pl.when(i + 2 < n_iter)
        def _():
            head_copy(i + 2).start()

        for u in range(UNROLL):
            mem = step(UNROLL * i + u, u, mem)
        return mem

    ln_x(0, 0)
    jax.lax.fori_loop(0, n_iter, iteration, mem0_ref[...].astype(F32))

    for s in range(n_seg, n_seg + G + 1):
        stages = ffn_stages(s)
        stages["down"](0)
        if s == n_seg:
            stages["ln_h"](0)
        if s < n_seg + G:
            stages["gate"](0)
            stages["up"](0)
        stages["write"](0)
    for g in range(n_grp):
        out_copy(g).wait()


@functools.partial(jax.jit, static_argnames=("A_seg_len",))
def pallas_sequential_preLN__memory_aug_recurrent_mem_tr__swiglu_ffn__prompt_kernel(
    A_x: jax.Array,
    A_mem0: jax.Array,
    A_Wq: jax.Array,
    A_Wk: jax.Array,
    A_Wv: jax.Array,
    A_Wo: jax.Array,
    A_seg_len: int,
    B_x: jax.Array,
    B_w_gate: jax.Array,
    B_w_up: jax.Array,
    B_w_down: jax.Array,
):
    del B_x
    B, S, D = A_x.shape
    _, H, Dh = A_Wq.shape
    M = A_mem0.shape[1]
    F = B_w_gate.shape[1]
    seg = int(A_seg_len)
    assert (B, S, H, Dh, M, seg) == (1, 2048, 32, 192, 8, 32)
    NP, PW, n_seg = H // 2, 2 * Dh, S // seg

    def rows_by_head(w):
        return jnp.transpose(w, (1, 2, 0)).reshape(H * Dh, D)

    hbm = pl.BlockSpec(memory_space=pl.ANY)
    out = pl.pallas_call(
        functools.partial(_kernel, S=S, D=D, H=H, Dh=Dh, M=M, seg=seg, F=F),
        out_shape=jax.ShapeDtypeStruct((S, D), A_x.dtype),
        in_specs=[hbm] * 9,
        out_specs=hbm,
        scratch_shapes=[
            pltpu.VMEM((n_seg, seg, D), BF16),
            pltpu.VMEM((n_seg * M, D), F32),
            pltpu.VMEM((2, seg, D), F32),
            pltpu.VMEM((NSTAGE, 3, PW, D), BF16),
            pltpu.VMEM((3 * NP, D // 2, PW), U32),
            pltpu.VMEM((NP, PW, D), BF16),
            pltpu.VMEM((G, D, F // G), BF16),
            pltpu.VMEM((G, D, F // G), BF16),
            pltpu.VMEM((G, F // G, D), BF16),
            pltpu.VMEM((n_seg * M, NP * sum(PRE_COLS)), F32),
            pltpu.VMEM((2, G * seg, D), F32),
            pltpu.VMEM((2, G * seg, D), F32),
            pltpu.VMEM((G * seg, F // G), F32),
            pltpu.VMEM((G * seg, D), F32),
            pltpu.VMEM((S, D), BF16),
            pltpu.VMEM((M, D), BF16),
            pltpu.SemaphoreType.DMA(()),
            pltpu.SemaphoreType.DMA((n_seg // SPC,)),
            pltpu.SemaphoreType.DMA((2,)),
            pltpu.SemaphoreType.DMA((NSTAGE, 3)),
            pltpu.SemaphoreType.DMA((NP,)),
            pltpu.SemaphoreType.DMA((3, G)),
            pltpu.SemaphoreType.DMA((S // (G * seg),)),
        ],
        compiler_params=pltpu.CompilerParams(vmem_limit_bytes=112 * 1024 * 1024),
    )(A_x.reshape(n_seg, seg, D), A_mem0.reshape(M, D),
      rows_by_head(A_Wq), rows_by_head(A_Wk), rows_by_head(A_Wv),
      A_Wo.reshape(H * Dh, D), B_w_gate, B_w_up, B_w_down)
    return out.reshape(B, S, D)
```
